```python
import os as _os
_os.environ.setdefault("JAX_PLATFORMS", "cpu")
import jax
import jax.numpy as jnp

def _softmax(x, axis=-1):
    return jax.nn.softmax(x, axis=axis)
def _gelu(x):
    return jax.nn.gelu(x, approximate=True)
def _silu(x):
    return jax.nn.silu(x)
def _sigmoid(x):
    return jax.nn.sigmoid(x)
def _layernorm(x, axis=-1, eps=1e-5):
    m = jnp.mean(x, axis=axis, keepdims=True)
    v = jnp.var(x, axis=axis, keepdims=True)
    return (x - m) / jnp.sqrt(v + eps)
def _scatter_add(tgt, idx, src, axis=0):
    return tgt.at[idx].add(src)
def _segment_sum(src, seg, n):
    return jax.ops.segment_sum(src, seg, n)
class _Rng:
    def __init__(self, key):
        self._k = key
    def _next(self):
        self._k, sub = jax.random.split(self._k)
        return sub
    def normal(self, shape):
        return jax.random.normal(self._next(), shape, dtype=jnp.bfloat16)
    def randint(self, lo, hi, shape):
        return jax.random.randint(self._next(), shape, lo, hi, dtype=jnp.int32)
    def uniform(self, shape, lo=0.0, hi=1.0):
        return jax.random.uniform(self._next(), shape, jnp.bfloat16, lo, hi)
    def permutation(self, n):
        return jax.random.permutation(self._next(), n)


kernel_name = 'standalone__mha_softmax__near_ridge'

def setup_inputs():
    _rng = _Rng(jax.random.key(int.from_bytes(__import__("os").urandom(4), "little")))
    _w = (lambda a: (lambda t: t.astype(jnp.bfloat16) if jnp.issubdtype(t.dtype, jnp.floating) else t)(jnp.asarray(a)))
    B, H, Sq, Sk, D = 8, 32, 496, 512, 192
    return {
        "q": _w((lambda *s: _rng.normal(s) * 0.05)(B, H, Sq, D)),
        "k": _w((lambda *s: _rng.normal(s) * 3.2)(B, H, Sk, D)),
        "v": _w((lambda *s: _rng.normal(s) * 0.05)(B, H, Sk, D)),
    }

def reference(q, k, v):
    scale = q.shape[-1] ** -0.5
    scores = jnp.einsum("bhqd,bhkd->bhqk", q, k) * scale
    p = _softmax(scores, axis=-1)
    return jnp.einsum("bhqk,bhkd->bhqd", p, v)
```

```python
import functools

import jax
import jax.numpy as jnp
from jax import lax
from jax.experimental import pallas as pl
from jax.experimental.pallas import tpu as pltpu

_LOG2E = 1.4426950408889634
_HEADS_PER_STEP = 8
_LANES = 512


def _kernel(qT_ref, kT_ref, vT_ref, oT_ref, *, scale, hb):
    c = scale * _LOG2E

    def qk(h):
        return lax.dot_general(
            kT_ref[h], qT_ref[h], (((0,), (0,)), ((), ())),
            preferred_element_type=jnp.float32)

    def softmax(sT):
        m = jnp.max(sT, axis=0, keepdims=True)
        p = jnp.exp2((sT - m) * c)
        l = jnp.sum(p, axis=0, keepdims=True)
        return p.astype(jnp.bfloat16), l

    def pv(h, p, l):
        oT = jnp.dot(vT_ref[h], p, preferred_element_type=jnp.float32)
        oT_ref[h] = (oT * (1.0 / l)).astype(oT_ref.dtype)

    s_next = qk(0)
    for h in range(hb):
        s = s_next
        if h + 1 < hb:
            s_next = qk(h + 1)
        p, l = softmax(s)
        pv(h, p, l)


@jax.jit
def pallas_standalone__mha_softmax__near_ridge_kernel(
    q: jax.Array,
    k: jax.Array,
    v: jax.Array,
):
    B, H, Sq, D = q.shape
    Sk = k.shape[2]
    hb = _HEADS_PER_STEP
    scale = D ** -0.5
    qT = jnp.swapaxes(q, 2, 3).reshape(B * H, D, Sq)
    kT = jnp.swapaxes(k, 2, 3).reshape(B * H, D, Sk)
    vT = jnp.swapaxes(v, 2, 3).reshape(B * H, D, Sk)
    oT = pl.pallas_call(
        functools.partial(_kernel, scale=scale, hb=hb),
        grid=(B * H // hb,),
        in_specs=[
            pl.BlockSpec((hb, D, _LANES), lambda i: (i, 0, 0)),
            pl.BlockSpec((hb, D, Sk), lambda i: (i, 0, 0)),
            pl.BlockSpec((hb, D, Sk), lambda i: (i, 0, 0)),
        ],
        out_specs=pl.BlockSpec((hb, D, _LANES), lambda i: (i, 0, 0)),
        out_shape=jax.ShapeDtypeStruct((B * H, D, Sq), q.dtype),
        compiler_params=pltpu.CompilerParams(
            dimension_semantics=("parallel",),
            vmem_limit_bytes=64 * 1024 * 1024,
            flags={"XLA_TPU_FORCE_LP_LLO_SCHEDULER": True},
        ),
    )(qT, kT, vT)
    return jnp.swapaxes(oT.reshape(B, H, D, Sq), 2, 3)
```

```python
import functools

import jax
import jax.numpy as jnp
from jax import lax
from jax.experimental import pallas as pl
from jax.experimental.pallas import tpu as pltpu

_LOG2E = 1.4426950408889634
_HEADS_PER_STEP = 8


def _kernel(qT_ref, kT_ref, vT_ref, oT_ref, *, scale, hb):
    c = scale * _LOG2E

    def qk(h):
        return lax.dot_general(
            qT_ref[h], kT_ref[h], (((0,), (0,)), ((), ())),
            preferred_element_type=jnp.float32)

    def softmax(s):
        m = jnp.max(s, axis=1, keepdims=True)
        p = jnp.exp2((s - m) * c)
        l = jnp.sum(p, axis=1, keepdims=True)
        return p.astype(jnp.bfloat16), l

    def pv(h, p, l):
        oT = lax.dot_general(
            vT_ref[h], p, (((1,), (1,)), ((), ())),
            preferred_element_type=jnp.float32)
        oT_ref[h] = (oT * (1.0 / l).T).astype(oT_ref.dtype)

    s = {0: qk(0)}
    pl_ = {}
    for h in range(hb + 1):
        if h + 1 < hb:
            s[h + 1] = qk(h + 1)
        if h - 1 >= 0:
            pv(h - 1, *pl_[h - 1])
        if h < hb:
            pl_[h] = softmax(s[h])


@jax.jit
def pallas_standalone__mha_softmax__near_ridge_kernel(
    q: jax.Array,
    k: jax.Array,
    v: jax.Array,
):
    B, H, Sq, D = q.shape
    Sk = k.shape[2]
    hb = _HEADS_PER_STEP
    scale = D ** -0.5
    qT = jnp.swapaxes(q, 2, 3).reshape(B * H, D, Sq)
    kT = jnp.swapaxes(k, 2, 3).reshape(B * H, D, Sk)
    vT = jnp.swapaxes(v, 2, 3).reshape(B * H, D, Sk)
    oT = pl.pallas_call(
        functools.partial(_kernel, scale=scale, hb=hb),
        grid=(B * H // hb,),
        in_specs=[
            pl.BlockSpec((hb, D, Sq), lambda i: (i, 0, 0)),
            pl.BlockSpec((hb, D, Sk), lambda i: (i, 0, 0)),
            pl.BlockSpec((hb, D, Sk), lambda i: (i, 0, 0)),
        ],
        out_specs=pl.BlockSpec((hb, D, Sq), lambda i: (i, 0, 0)),
        out_shape=jax.ShapeDtypeStruct((B * H, D, Sq), q.dtype),
        compiler_params=pltpu.CompilerParams(
            dimension_semantics=("parallel",),
            vmem_limit_bytes=64 * 1024 * 1024,
        ),
    )(qT, kT, vT)
    return jnp.swapaxes(oT.reshape(B, H, D, Sq), 2, 3)
```

```python
import functools

import jax
import jax.numpy as jnp
from jax import lax
from jax.experimental import pallas as pl
from jax.experimental.pallas import tpu as pltpu

_LOG2E = 1.4426950408889634

_HEAD_GROUPS = (2, 2)
_RAMP_G, _RAMP_N = 4, 3
_G = 8
_LOOKAHEAD = 3
_IN_REGIONS = _LOOKAHEAD + 1
_OUT_REGIONS = 2
_OUT_CHUNK = 4


def _kernel(q_hbm, k_hbm, v_hbm, o_hbm, qb, kb, vb, ob, s_st, p_st, r_st,
            sin, sout, *, scale, n_heads):
    c = scale * _LOG2E
    G, G1, n1 = _G, _RAMP_G, _RAMP_N
    R, RO, L = _IN_REGIONS, _OUT_REGIONS, _LOOKAHEAD
    nhs = sum(_HEAD_GROUPS)
    nh = nhs + G1 * n1
    nmain = (n_heads - nh) // G
    sem_ramp = len(_HEAD_GROUPS)
    sem_main = sem_ramp + n1
    out0 = nh - 2
    out_tail = out0 + RO * G

    def in_copies(a, n, slot, si):
        return (
            pltpu.make_async_copy(
                q_hbm.at[pl.ds(a, n)], qb.at[pl.ds(slot, n)], sin.at[0, si]),
            pltpu.make_async_copy(
                k_hbm.at[pl.ds(a, n)], kb.at[pl.ds(slot, n)], sin.at[1, si]),
            pltpu.make_async_copy(
                v_hbm.at[pl.ds(a, n)], vb.at[pl.ds(slot, n)], sin.at[2, si]),
        )

    def start_in(a, n, slot, si):
        for cp in in_copies(a, n, slot, si):
            cp.start()

    def wait_in(a, n, slot, si):
        for cp in in_copies(a, n, slot, si):
            cp.wait()

    def out_copy(a, n, slot, si):
        return pltpu.make_async_copy(
            ob.at[pl.ds(slot, n)], o_hbm.at[pl.ds(a, n)], sout.at[si])

    def qk(slot):
        return lax.dot_general(
            qb[slot], kb[slot], (((0,), (0,)), ((), ())),
            preferred_element_type=jnp.float32)

    def softmax(s, carried=False):
        m = jnp.max(s, axis=1, keepdims=True)
        p = jnp.exp2((s - m) * c)
        l = jnp.sum(p, axis=1, keepdims=True)
        r = 1.0 / l.T if carried else (1.0 / l).T
        return p, r

    def pv(slot, oslot, p, r):
        oT = lax.dot_general(
            vb[slot], p.astype(jnp.bfloat16), (((1,), (1,)), ((), ())),
            preferred_element_type=jnp.float32)
        ob[oslot] = (oT * r).astype(ob.dtype)

    def save_state(s, p, r):
        s_st[...] = s
        p_st[...] = p
        r_st[...] = r

    a = 0
    group_of = {}
    for gi, n in enumerate(_HEAD_GROUPS):
        start_in(a, n, a, gi)
        group_of[a] = (gi, n)
        a += n
    for g in range(n1):
        start_in(nhs + g * G1, G1, nhs + g * G1, sem_ramp + g)
    for g in range(min(L, nmain)):
        start_in(nh + g * G, G, nh + g * G, sem_main + g)

    S, P = {}, {}
    for h in range(-1, nhs - 1):
        if (h + 1) in group_of:
            gi, n = group_of[h + 1]
            wait_in(h + 1, n, h + 1, gi)
        if h - 1 >= 0:
            pv(h - 1, h - 1, *P.pop(h - 1))
        if h >= 0:
            P[h] = softmax(S.pop(h), carried=(h == nhs - 2))
        S[h + 1] = qk(h + 1)
    save_state(S.pop(nhs - 1), *P.pop(nhs - 2))

    def segment(n, a, base, pbase, obase, osem, chunk, prefetch=None):
        S = {-1: s_st[...]}
        P = {-2: (p_st[...], r_st[...])}
        for i in range(-1, n - 1):
            j = i - 1
            pv(pbase + j + 2 if j < 0 else base + j, obase + j + 2, *P.pop(j))
            done = j + 3
            if chunk and done % chunk == 0:
                p0 = done - chunk
                out_copy(a - 2 + p0, chunk, obase + p0, osem).start()
            P[i] = softmax(S.pop(i), carried=(i == n - 2))
            S[i + 1] = qk(base + i + 1)
            if prefetch is not None and i == 0:
                prefetch()
        save_state(S.pop(n - 1), *P.pop(n - 2))

    def ramp_body(g, carry):
        a = nhs + g * G1
        wait_in(a, G1, a, sem_ramp + g)
        segment(G1, a, a, a - 2, a - 2, 0, 0)
        return carry

    lax.fori_loop(0, n1, ramp_body, 0)
    out_copy(0, nh - 2, 0, 0).start()

    def main_body(g, carry):
        r, ro = g % R, g % RO
        rp = (g + R - 1) % R
        a = nh + g * G
        wait_in(a, G, nh + r * G, sem_main + r)

        @pl.when(g >= RO)
        def _():
            out_copy(a - 2 - RO * G, G, out0 + ro * G, 1 + ro).wait()

        def prefetch():
            gn = g + L

            @pl.when(gn < nmain)
            def _():
                start_in(nh + gn * G, G, nh + (gn % R) * G, sem_main + gn % R)

        pbase = jnp.where(g == 0, nh - 2, nh + rp * G + G - 2)
        segment(G, a, nh + r * G, pbase, out0 + ro * G, 1 + ro, _OUT_CHUNK,
                prefetch)
        return carry

    lax.fori_loop(0, nmain, main_body, 0)

    last = nh + ((nmain - 1) % R) * G
    pv(last + G - 2, out_tail, p_st[...], r_st[...])
    out_copy(n_heads - 2, 1, out_tail, 1 + RO).start()
    pv(last + G - 1, out_tail + 1, *softmax(s_st[...]))
    out_copy(n_heads - 1, 1, out_tail + 1, 1 + RO).start()

    out_copy(0, nh - 2, 0, 0).wait()
    for g in range(max(nmain - RO, 0), nmain):
        out_copy(nh + g * G - 2, G, out0 + (g % RO) * G, 1 + g % RO).wait()
    out_copy(n_heads - 2, 2, out_tail, 1 + RO).wait()


@jax.jit
def pallas_standalone__mha_softmax__near_ridge_kernel(
    q: jax.Array,
    k: jax.Array,
    v: jax.Array,
):
    B, H, Sq, D = q.shape
    Sk = k.shape[2]
    n_heads = B * H
    scale = D ** -0.5
    nh = sum(_HEAD_GROUPS) + _RAMP_G * _RAMP_N
    assert (n_heads - nh) % _G == 0 and n_heads - nh >= _G * _LOOKAHEAD

    qT = jnp.swapaxes(q, 2, 3).reshape(n_heads, D, Sq)
    kT = jnp.swapaxes(k, 2, 3).reshape(n_heads, D, Sk)
    vT = jnp.swapaxes(v, 2, 3).reshape(n_heads, D, Sk)

    n_in = nh + _IN_REGIONS * _G
    n_out = nh + _OUT_REGIONS * _G
    oT = pl.pallas_call(
        functools.partial(_kernel, scale=scale, n_heads=n_heads),
        in_specs=[pl.BlockSpec(memory_space=pl.ANY)] * 3,
        out_specs=pl.BlockSpec(memory_space=pl.ANY),
        out_shape=jax.ShapeDtypeStruct((n_heads, D, Sq), q.dtype),
        scratch_shapes=[
            pltpu.VMEM((n_in, D, Sq), q.dtype),
            pltpu.VMEM((n_in, D, Sk), k.dtype),
            pltpu.VMEM((n_in, D, Sk), v.dtype),
            pltpu.VMEM((n_out, D, Sq), q.dtype),
            pltpu.VMEM((Sq, Sk), jnp.float32),
            pltpu.VMEM((Sq, Sk), jnp.float32),
            pltpu.VMEM((1, Sq), jnp.float32),
            pltpu.SemaphoreType.DMA(
                (3, len(_HEAD_GROUPS) + _RAMP_N + _IN_REGIONS)),
            pltpu.SemaphoreType.DMA((2 + _OUT_REGIONS,)),
        ],
        compiler_params=pltpu.CompilerParams(
            vmem_limit_bytes=100 * 1024 * 1024,
            disable_bounds_checks=True,
        ),
    )(qT, kT, vT)
    return jnp.swapaxes(oT.reshape(B, H, D, Sq), 2, 3)
```

```python
import functools

import jax
import jax.numpy as jnp
from jax import lax
from jax.experimental import pallas as pl
from jax.experimental.pallas import tpu as pltpu

_LOG2E = 1.4426950408889634

_HEAD_GROUPS = (2, 2)
_RAMP_G, _RAMP_N = 4, 3
_G = 8
_LOOKAHEAD = 3
_IN_REGIONS = _LOOKAHEAD + 1
_OUT_REGIONS = 2
_OUT_CHUNK = 4
_PREFETCH_STEP = 3
_MAIN_ORDER = ("peq", "epq", "eqp", "epq", "pqe", "pqe", "qpe", "qpe")
_MAIN_RECIP = ("col", "col", "col", "col", "col", "row", "late", "col")


def _kernel(q_hbm, k_hbm, v_hbm, o_hbm, qb, kb, vb, ob, s_st, p_st, r_st,
            sin, sout, *, scale, n_heads):
    c = scale * _LOG2E
    G, G1, n1 = _G, _RAMP_G, _RAMP_N
    R, RO, L = _IN_REGIONS, _OUT_REGIONS, _LOOKAHEAD
    nhs = sum(_HEAD_GROUPS)
    nh = nhs + G1 * n1
    nmain = (n_heads - nh) // G
    sem_ramp = len(_HEAD_GROUPS)
    sem_main = sem_ramp + n1
    out0 = nh - 2
    out_tail = out0 + RO * G

    def in_copies(a, n, slot, si):
        return (
            pltpu.make_async_copy(
                q_hbm.at[pl.ds(a, n)], qb.at[pl.ds(slot, n)], sin.at[0, si]),
            pltpu.make_async_copy(
                k_hbm.at[pl.ds(a, n)], kb.at[pl.ds(slot, n)], sin.at[1, si]),
            pltpu.make_async_copy(
                v_hbm.at[pl.ds(a, n)], vb.at[pl.ds(slot, n)], sin.at[2, si]),
        )

    def start_in(a, n, slot, si):
        for cp in in_copies(a, n, slot, si):
            cp.start()

    def wait_in(a, n, slot, si):
        for cp in in_copies(a, n, slot, si):
            cp.wait()

    def out_copy(a, n, slot, si):
        return pltpu.make_async_copy(
            ob.at[pl.ds(slot, n)], o_hbm.at[pl.ds(a, n)], sout.at[si])

    def qk(slot):
        return lax.dot_general(
            qb[slot], kb[slot], (((0,), (0,)), ((), ())),
            preferred_element_type=jnp.float32)

    def recip(l):
        r = pl.reciprocal(l, approx=True)
        return r * (2.0 - l * r)

    def softmax(s, mode="col"):
        m = jnp.max(s, axis=1, keepdims=True)
        p = jnp.exp2((s - m) * c)
        l = jnp.sum(p, axis=1, keepdims=True)
        if mode == "col":
            return p, recip(l).T
        if mode == "row":
            return p, recip(l.T)
        return p, l.T

    def pv(slot, oslot, p, r, mode="col"):
        oT = lax.dot_general(
            vb[slot], p.astype(jnp.bfloat16), (((1,), (1,)), ((), ())),
            preferred_element_type=jnp.float32)
        if mode == "late":
            r = recip(r)
        ob[oslot] = (oT * r).astype(ob.dtype)

    def save_state(s, p, r):
        s_st[...] = s
        p_st[...] = p
        r_st[...] = r

    a = 0
    group_of = {}
    for gi, n in enumerate(_HEAD_GROUPS):
        start_in(a, n, a, gi)
        group_of[a] = (gi, n)
        a += n
    for g in range(n1):
        start_in(nhs + g * G1, G1, nhs + g * G1, sem_ramp + g)
    for g in range(min(L, nmain)):
        start_in(nh + g * G, G, nh + g * G, sem_main + g)

    S, P = {}, {}
    for h in range(-1, nhs - 1):
        if (h + 1) in group_of:
            gi, n = group_of[h + 1]
            wait_in(h + 1, n, h + 1, gi)
        if h - 1 >= 0:
            pv(h - 1, h - 1, *P.pop(h - 1))
        if h >= 0:
            P[h] = softmax(S.pop(h))
        S[h + 1] = qk(h + 1)
    save_state(S.pop(nhs - 1), *P.pop(nhs - 2))

    def segment(n, a, base, pbase, obase, osem, chunk, orders, modes,
                prefetch=None):
        S = {-1: s_st[...]}
        P = {-2: (p_st[...], r_st[...])}

        def step_pv(i):
            j = i - 1
            pv(pbase + j + 2 if j < 0 else base + j, obase + j + 2, *P.pop(j),
               mode=modes[j + 1] if j >= -1 else modes[-1])
            done = j + 3
            if chunk and done % chunk == 0:
                p0 = done - chunk
                out_copy(a - 2 + p0, chunk, obase + p0, osem).start()

        def step_softmax(i):
            P[i] = softmax(S.pop(i), modes[i + 1])

        def step_qk(i):
            S[i + 1] = qk(base + i + 1)

        for i in range(-1, n - 1):
            for piece in orders[i + 1]:
                {"p": step_pv, "e": step_softmax, "q": step_qk}[piece](i)
            if prefetch is not None and i == _PREFETCH_STEP:
                prefetch()
        save_state(S.pop(n - 1), *P.pop(n - 2))

    def ramp_body(g, carry):
        a = nhs + g * G1
        wait_in(a, G1, a, sem_ramp + g)
        segment(G1, a, a, a - 2, a - 2, 0, 0, ("peq",) * G1, ("col",) * G1)
        return carry

    lax.fori_loop(0, n1, ramp_body, 0)
    out_copy(0, nh - 2, 0, 0).start()

    def main_body(g, carry):
        r, ro = g % R, g % RO
        rp = (g + R - 1) % R
        a = nh + g * G
        wait_in(a, G, nh + r * G, sem_main + r)

        @pl.when(g >= RO)
        def _():
            out_copy(a - 2 - RO * G, G, out0 + ro * G, 1 + ro).wait()

        def prefetch():
            gn = g + L

            @pl.when(gn < nmain)
            def _():
                start_in(nh + gn * G, G, nh + (gn % R) * G, sem_main + gn % R)

        pbase = jnp.where(g == 0, nh - 2, nh + rp * G + G - 2)
        segment(G, a, nh + r * G, pbase, out0 + ro * G, 1 + ro, _OUT_CHUNK,
                _MAIN_ORDER, _MAIN_RECIP, prefetch)
        return carry

    lax.fori_loop(0, nmain, main_body, 0)

    last = nh + ((nmain - 1) % R) * G
    pv(last + G - 2, out_tail, p_st[...], r_st[...])
    out_copy(n_heads - 2, 1, out_tail, 1 + RO).start()
    pv(last + G - 1, out_tail + 1, *softmax(s_st[...], "row"))
    out_copy(n_heads - 1, 1, out_tail + 1, 1 + RO).start()

    out_copy(0, nh - 2, 0, 0).wait()
    for g in range(max(nmain - RO, 0), nmain):
        out_copy(nh + g * G - 2, G, out0 + (g % RO) * G, 1 + g % RO).wait()
    out_copy(n_heads - 2, 2, out_tail, 1 + RO).wait()


@jax.jit
def pallas_standalone__mha_softmax__near_ridge_kernel(
    q: jax.Array,
    k: jax.Array,
    v: jax.Array,
):
    B, H, Sq, D = q.shape
    Sk = k.shape[2]
    n_heads = B * H
    scale = D ** -0.5
    nh = sum(_HEAD_GROUPS) + _RAMP_G * _RAMP_N
    assert (n_heads - nh) % _G == 0 and n_heads - nh >= _G * _LOOKAHEAD

    qT = jnp.swapaxes(q, 2, 3).reshape(n_heads, D, Sq)
    kT = jnp.swapaxes(k, 2, 3).reshape(n_heads, D, Sk)
    vT = jnp.swapaxes(v, 2, 3).reshape(n_heads, D, Sk)

    n_in = nh + _IN_REGIONS * _G
    n_out = nh + _OUT_REGIONS * _G
    oT = pl.pallas_call(
        functools.partial(_kernel, scale=scale, n_heads=n_heads),
        in_specs=[pl.BlockSpec(memory_space=pl.ANY)] * 3,
        out_specs=pl.BlockSpec(memory_space=pl.ANY),
        out_shape=jax.ShapeDtypeStruct((n_heads, D, Sq), q.dtype),
        scratch_shapes=[
            pltpu.VMEM((n_in, D, Sq), q.dtype),
            pltpu.VMEM((n_in, D, Sk), k.dtype),
            pltpu.VMEM((n_in, D, Sk), v.dtype),
            pltpu.VMEM((n_out, D, Sq), q.dtype),
            pltpu.VMEM((Sq, Sk), jnp.float32),
            pltpu.VMEM((Sq, Sk), jnp.float32),
            pltpu.VMEM((1, Sq), jnp.float32),
            pltpu.SemaphoreType.DMA(
                (3, len(_HEAD_GROUPS) + _RAMP_N + _IN_REGIONS)),
            pltpu.SemaphoreType.DMA((2 + _OUT_REGIONS,)),
        ],
        compiler_params=pltpu.CompilerParams(
            vmem_limit_bytes=100 * 1024 * 1024,
            disable_bounds_checks=True,
        ),
    )(qT, kT, vT)
    return jnp.swapaxes(oT.reshape(B, H, D, Sq), 2, 3)
```

```python
import functools

import jax
import jax.numpy as jnp
from jax import lax
from jax.experimental import pallas as pl
from jax.experimental.pallas import tpu as pltpu

_LOG2E = 1.4426950408889634

_FIRST = 2
_RAMP = ((2, 1), (4, 3))
_G = 8
_LOOKAHEAD = 3
_IN_REGIONS = _LOOKAHEAD + 1
_OUT_REGIONS = 2
_OUT_CHUNK = 4
_PREFETCH_STEP = 3
_MAIN_ORDER = ("peq", "epq", "eqp", "epq", "pqe", "pqe", "qpe", "qpe")
_MAIN_RECIP = ("col", "col", "col", "col", "col", "row", "late", "col")


def _kernel(q_hbm, k_hbm, v_hbm, o_hbm, qb, kb, vb, ob, s_st, p_st, r_st,
            sin, sout, *, scale, n_heads):
    c = scale * _LOG2E
    G, R, RO, L = _G, _IN_REGIONS, _OUT_REGIONS, _LOOKAHEAD
    nh = _FIRST + sum(n * cnt for n, cnt in _RAMP)
    nmain = (n_heads - nh) // G
    sem_main = 1 + sum(cnt for _, cnt in _RAMP)
    sem_last = sem_main + R
    slot_last = nh + R * G
    out0 = nh - 2
    out_last = out0 + RO * G

    def in_copy(kind, a, n, slot, si):
        src, dst = ((q_hbm, qb), (k_hbm, kb), (v_hbm, vb))[kind]
        return pltpu.make_async_copy(
            src.at[pl.ds(a, n)], dst.at[pl.ds(slot, n)], sin.at[kind, si])

    def in_group(a, n, slot, si):
        return (in_copy(0, a, n, slot, si), in_copy(1, a, n, slot, si),
                in_copy(2, a - 2, n, slot, si))

    def out_copy(a, n, slot, si):
        return pltpu.make_async_copy(
            ob.at[pl.ds(slot, n)], o_hbm.at[pl.ds(a, n)], sout.at[si])

    def qk(slot):
        return lax.dot_general(
            qb[slot], kb[slot], (((0,), (0,)), ((), ())),
            preferred_element_type=jnp.float32)

    def recip(l):
        r = pltpu.reciprocal(l, approx=True)
        return r * (2.0 - l * r)

    def softmax(s, mode="col"):
        m = jnp.max(s, axis=1, keepdims=True)
        p = jnp.exp2((s - m) * c)
        l = jnp.sum(p, axis=1, keepdims=True)
        if mode == "col":
            return p, recip(l).T
        if mode == "row":
            return p, recip(l.T)
        return p, l.T

    def pv(slot, oslot, p, r, mode="col"):
        oT = lax.dot_general(
            vb[slot], p.astype(jnp.bfloat16), (((1,), (1,)), ((), ())),
            preferred_element_type=jnp.float32)
        if mode == "late":
            r = recip(r)
        ob[oslot] = (oT * r).astype(ob.dtype)

    def save_state(s, p, r):
        s_st[...] = s
        p_st[...] = p
        r_st[...] = r

    first = (in_copy(0, 0, _FIRST, 0, 0), in_copy(1, 0, _FIRST, 0, 0))
    for cp in first:
        cp.start()
    a, si = _FIRST, 1
    for n, cnt in _RAMP:
        for _ in range(cnt):
            for cp in in_group(a, n, a, si):
                cp.start()
            a, si = a + n, si + 1
    for g in range(min(L, nmain)):
        for cp in in_group(nh + g * G, G, nh + g * G, sem_main + g):
            cp.start()

    for cp in first:
        cp.wait()
    s0 = qk(0)
    s1 = qk(1)
    save_state(s1, *softmax(s0))

    def segment(n, a, base, obase, osem, chunk, orders, modes, prefetch=None):
        S = {-1: s_st[...]}
        P = {-2: (p_st[...], r_st[...])}

        def step_pv(i):
            j = i - 1
            pv(base + j + 2, obase + j + 2, *P.pop(j),
               mode=modes[j + 1] if j >= -1 else modes[-1])
            done = j + 3
            if chunk and done % chunk == 0:
                p0 = done - chunk
                out_copy(a - 2 + p0, chunk, obase + p0, osem).start()

        def step_softmax(i):
            P[i] = softmax(S.pop(i), modes[i + 1])

        def step_qk(i):
            S[i + 1] = qk(base + i + 1)

        for i in range(-1, n - 1):
            for piece in orders[i + 1]:
                {"p": step_pv, "e": step_softmax, "q": step_qk}[piece](i)
            if prefetch is not None and i == _PREFETCH_STEP:
                prefetch()
        save_state(S.pop(n - 1), *P.pop(n - 2))

    a0, si0 = _FIRST, 1
    for n, cnt in _RAMP:

        def ramp_body(g, carry, n=n, a0=a0, si0=si0):
            a = a0 + g * n
            for cp in in_group(a, n, a, si0 + g):
                cp.wait()
            segment(n, a, a, a - 2, 0, 0, ("peq",) * n, ("col",) * n)
            return carry

        lax.fori_loop(0, cnt, ramp_body, 0)
        a0, si0 = a0 + n * cnt, si0 + cnt
    out_copy(0, nh - 2, 0, 0).start()

    def main_body(g, carry):
        r, ro = g % R, g % RO
        a = nh + g * G
        for cp in in_group(a, G, nh + r * G, sem_main + r):
            cp.wait()

        @pl.when(g >= RO)
        def _():
            out_copy(a - 2 - RO * G, G, out0 + ro * G, 1 + ro).wait()

        def prefetch():
            gn = g + L

            @pl.when(gn < nmain)
            def _():
                rn = gn % R
                for cp in in_group(nh + gn * G, G, nh + rn * G, sem_main + rn):
                    cp.start()

            @pl.when(gn == nmain)
            def _():
                in_copy(2, n_heads - 2, 2, slot_last, sem_last).start()

        segment(G, a, nh + r * G, out0 + ro * G, 1 + ro, _OUT_CHUNK,
                _MAIN_ORDER, _MAIN_RECIP, prefetch)
        return carry

    lax.fori_loop(0, nmain, main_body, 0)

    in_copy(2, n_heads - 2, 2, slot_last, sem_last).wait()
    pv(slot_last, out_last, p_st[...], r_st[...], _MAIN_RECIP[-1])
    out_copy(n_heads - 2, 1, out_last, 1 + RO).start()
    pv(slot_last + 1, out_last + 1, *softmax(s_st[...], "row"), mode="row")
    out_copy(n_heads - 1, 1, out_last + 1, 1 + RO).start()

    out_copy(0, nh - 2, 0, 0).wait()
    for g in range(max(nmain - RO, 0), nmain):
        out_copy(nh + g * G - 2, G, out0 + (g % RO) * G, 1 + g % RO).wait()
    out_copy(n_heads - 2, 2, out_last, 1 + RO).wait()


@jax.jit
def pallas_standalone__mha_softmax__near_ridge_kernel(
    q: jax.Array,
    k: jax.Array,
    v: jax.Array,
):
    B, H, Sq, D = q.shape
    Sk = k.shape[2]
    n_heads = B * H
    scale = D ** -0.5
    nh = _FIRST + sum(n * cnt for n, cnt in _RAMP)
    assert (n_heads - nh) % _G == 0 and n_heads - nh >= _G * _LOOKAHEAD

    qT = jnp.swapaxes(q, 2, 3).reshape(n_heads, D, Sq)
    kT = jnp.swapaxes(k, 2, 3).reshape(n_heads, D, Sk)
    vT = jnp.swapaxes(v, 2, 3).reshape(n_heads, D, Sk)

    n_in = nh + _IN_REGIONS * _G
    n_out = nh + _OUT_REGIONS * _G
    n_sem_in = 1 + sum(cnt for _, cnt in _RAMP) + _IN_REGIONS + 1
    oT = pl.pallas_call(
        functools.partial(_kernel, scale=scale, n_heads=n_heads),
        in_specs=[pl.BlockSpec(memory_space=pl.ANY)] * 3,
        out_specs=pl.BlockSpec(memory_space=pl.ANY),
        out_shape=jax.ShapeDtypeStruct((n_heads, D, Sq), q.dtype),
        scratch_shapes=[
            pltpu.VMEM((n_in, D, Sq), q.dtype),
            pltpu.VMEM((n_in, D, Sk), k.dtype),
            pltpu.VMEM((n_in + 2, D, Sk), v.dtype),
            pltpu.VMEM((n_out, D, Sq), q.dtype),
            pltpu.VMEM((Sq, Sk), jnp.float32),
            pltpu.VMEM((Sq, Sk), jnp.float32),
            pltpu.VMEM((1, Sq), jnp.float32),
            pltpu.SemaphoreType.DMA((3, n_sem_in)),
            pltpu.SemaphoreType.DMA((2 + _OUT_REGIONS,)),
        ],
        compiler_params=pltpu.CompilerParams(
            vmem_limit_bytes=100 * 1024 * 1024,
            disable_bounds_checks=True,
        ),
    )(qT, kT, vT)
    return jnp.swapaxes(oT.reshape(B, H, D, Sq), 2, 3)
```

```python
import functools

import jax
import jax.numpy as jnp
from jax import lax
from jax.experimental import pallas as pl
from jax.experimental.pallas import tpu as pltpu

_LOG2E = 1.4426950408889634

_FIRST = 2
_LOOKAHEAD = 3
_IN_REGIONS = _LOOKAHEAD + 1
_OUT_REGIONS = 2
_OUT_CHUNK = 5
_PREFETCH_STEP = 2

_CARRIED = "late"
_MAIN = (
    ("epq", "col", 4), ("qep", "col", 2), ("qpe", "col", 1), ("qep", "col", 2),
    ("qpe", "col", 4), ("eqp", "col", 4), ("qpe", "row", 2), ("qpe", "late", 1),
    ("epq", "row", 2), ("qpe", _CARRIED, 2),
)
_RAMP = (
    ((("pqe", "col", 1), ("epq", _CARRIED, 1)), 2),
    ((("epq", "col", 1), ("peq", "row", 1), ("qpe", "row", 1),
      ("qpe", _CARRIED, 1)), 5),
)
_G = len(_MAIN)


def _kernel(q_hbm, k_hbm, v_hbm, o_hbm, qb, kb, vb, ob, s_st, p_st, r_st,
            sin, sout, *, scale, n_heads):
    c = scale * _LOG2E
    G, R, RO, L = _G, _IN_REGIONS, _OUT_REGIONS, _LOOKAHEAD
    nh = _FIRST + sum(len(seg) * cnt for seg, cnt in _RAMP)
    nmain = (n_heads - nh) // G
    sem_main = 1 + sum(cnt for _, cnt in _RAMP)
    sem_last = sem_main + R
    slot_last = nh + R * G
    out0 = nh - 2
    out_last = out0 + RO * G

    def in_copy(kind, a, n, slot, si):
        src, dst = ((q_hbm, qb), (k_hbm, kb), (v_hbm, vb))[kind]
        return pltpu.make_async_copy(
            src.at[pl.ds(a, n)], dst.at[pl.ds(slot, n)], sin.at[kind, si])

    def in_group(a, n, slot, si):
        return (in_copy(0, a, n, slot, si), in_copy(1, a, n, slot, si),
                in_copy(2, a - 2, n, slot, si))

    def out_copy(a, n, slot, si):
        return pltpu.make_async_copy(
            ob.at[pl.ds(slot, n)], o_hbm.at[pl.ds(a, n)], sout.at[si])

    def qk(slot):
        return lax.dot_general(
            qb[slot], kb[slot], (((0,), (0,)), ((), ())),
            preferred_element_type=jnp.float32)

    def recip(l):
        r = pltpu.reciprocal(l, approx=True)
        return r * (2.0 - l * r)

    def softmax(s, mode):
        m = jnp.max(s, axis=1, keepdims=True)
        p = jnp.exp2((s - m) * c)
        l = jnp.sum(p, axis=1, keepdims=True)
        if mode == "col":
            return p, recip(l).T
        if mode == "row":
            return p, recip(l.T)
        return p, l.T

    def pv(slot, oslot, p, r, mode, split=1):
        if mode == "late":
            r = recip(r)
        sq = p.shape[0]
        w = sq if split == 1 else pl.cdiv(sq, 128 * split) * 128
        for q0 in range(0, sq, w):
            q1 = min(q0 + w, sq)
            oT = lax.dot_general(
                vb[slot], p[q0:q1].astype(jnp.bfloat16),
                (((1,), (1,)), ((), ())), preferred_element_type=jnp.float32)
            ob[oslot, :, q0:q1] = (oT * r[:, q0:q1]).astype(ob.dtype)

    def save_state(s, p, r):
        s_st[...] = s
        p_st[...] = p
        r_st[...] = r

    first = (in_copy(0, 0, _FIRST, 0, 0), in_copy(1, 0, _FIRST, 0, 0))
    for cp in first:
        cp.start()
    a, si = _FIRST, 1
    for seg, cnt in _RAMP:
        n = len(seg)
        for _ in range(cnt):
            for cp in in_group(a, n, a, si):
                cp.start()
            a, si = a + n, si + 1
    for g in range(min(L, nmain)):
        for cp in in_group(nh + g * G, G, nh + g * G, sem_main + g):
            cp.start()

    for cp in first:
        cp.wait()
    s0 = qk(0)
    s1 = qk(1)
    save_state(s1, *softmax(s0, _CARRIED))

    def segment(steps, a, base, obase, osem, chunk=0, prefetch=None):
        n = len(steps)
        S, P = {}, {}

        def step_pv(i):
            j = i - 1
            if j == -2:
                p, r, mode = p_st[...], r_st[...], _CARRIED
            else:
                (p, r), mode = P.pop(j), steps[j + 1][1]
            pv(base + j + 2, obase + j + 2, p, r, mode, steps[i + 1][2])
            done = j + 3
            if chunk and done % chunk == 0:
                p0 = done - chunk
                out_copy(a - 2 + p0, chunk, obase + p0, osem).start()

        def step_softmax(i):
            s = s_st[...] if i == -1 else S.pop(i)
            P[i] = softmax(s, steps[i + 1][1])

        def step_qk(i):
            S[i + 1] = qk(base + i + 1)

        for i in range(-1, n - 1):
            for piece in steps[i + 1][0]:
                {"p": step_pv, "e": step_softmax, "q": step_qk}[piece](i)
            if prefetch is not None and i == _PREFETCH_STEP:
                prefetch()
        save_state(S.pop(n - 1), *P.pop(n - 2))

    a0, si0 = _FIRST, 1
    for seg, cnt in _RAMP:

        def ramp_body(g, carry, seg=seg, a0=a0, si0=si0):
            a = a0 + g * len(seg)
            for cp in in_group(a, len(seg), a, si0 + g):
                cp.wait()
            segment(seg, a, a, a - 2, 0)
            return carry

        lax.fori_loop(0, cnt, ramp_body, 0)
        a0, si0 = a0 + len(seg) * cnt, si0 + cnt
    out_copy(0, nh - 2, 0, 0).start()

    def main_body(g, carry):
        r, ro = g % R, g % RO
        a = nh + g * G
        for cp in in_group(a, G, nh + r * G, sem_main + r):
            cp.wait()

        @pl.when(g >= RO)
        def _():
            out_copy(a - 2 - RO * G, G, out0 + ro * G, 1 + ro).wait()

        def prefetch():
            gn = g + L

            @pl.when(gn < nmain)
            def _():
                rn = gn % R
                for cp in in_group(nh + gn * G, G, nh + rn * G, sem_main + rn):
                    cp.start()

            @pl.when(gn == nmain)
            def _():
                in_copy(2, n_heads - 2, 2, slot_last, sem_last).start()

        segment(_MAIN, a, nh + r * G, out0 + ro * G, 1 + ro, _OUT_CHUNK,
                prefetch)
        return carry

    lax.fori_loop(0, nmain, main_body, 0)

    in_copy(2, n_heads - 2, 2, slot_last, sem_last).wait()
    pv(slot_last, out_last, p_st[...], r_st[...], _CARRIED)
    out_copy(n_heads - 2, 1, out_last, 1 + RO).start()
    pv(slot_last + 1, out_last + 1, *softmax(s_st[...], "row"), "row")
    out_copy(n_heads - 1, 1, out_last + 1, 1 + RO).start()

    out_copy(0, nh - 2, 0, 0).wait()
    for g in range(max(nmain - RO, 0), nmain):
        out_copy(nh + g * G - 2, G, out0 + (g % RO) * G, 1 + g % RO).wait()
    out_copy(n_heads - 2, 2, out_last, 1 + RO).wait()


@jax.jit
def pallas_standalone__mha_softmax__near_ridge_kernel(
    q: jax.Array,
    k: jax.Array,
    v: jax.Array,
):
    B, H, Sq, D = q.shape
    Sk = k.shape[2]
    n_heads = B * H
    scale = D ** -0.5
    nh = _FIRST + sum(len(seg) * cnt for seg, cnt in _RAMP)
    assert (n_heads - nh) % _G == 0 and n_heads - nh >= _G * _LOOKAHEAD

    qT = jnp.swapaxes(q, 2, 3).reshape(n_heads, D, Sq)
    kT = jnp.swapaxes(k, 2, 3).reshape(n_heads, D, Sk)
    vT = jnp.swapaxes(v, 2, 3).reshape(n_heads, D, Sk)

    n_in = nh + _IN_REGIONS * _G
    n_out = nh + _OUT_REGIONS * _G
    n_sem_in = 1 + sum(cnt for _, cnt in _RAMP) + _IN_REGIONS + 1
    oT = pl.pallas_call(
        functools.partial(_kernel, scale=scale, n_heads=n_heads),
        in_specs=[pl.BlockSpec(memory_space=pl.ANY)] * 3,
        out_specs=pl.BlockSpec(memory_space=pl.ANY),
        out_shape=jax.ShapeDtypeStruct((n_heads, D, Sq), q.dtype),
        scratch_shapes=[
            pltpu.VMEM((n_in, D, Sq), q.dtype),
            pltpu.VMEM((n_in, D, Sk), k.dtype),
            pltpu.VMEM((n_in + 2, D, Sk), v.dtype),
            pltpu.VMEM((n_out, D, Sq), q.dtype),
            pltpu.VMEM((Sq, Sk), jnp.float32),
            pltpu.VMEM((Sq, Sk), jnp.float32),
            pltpu.VMEM((1, Sq), jnp.float32),
            pltpu.SemaphoreType.DMA((3, n_sem_in)),
            pltpu.SemaphoreType.DMA((2 + _OUT_REGIONS,)),
        ],
        compiler_params=pltpu.CompilerParams(
            vmem_limit_bytes=100 * 1024 * 1024,
            disable_bounds_checks=True,
        ),
    )(qT, kT, vT)
    return jnp.swapaxes(oT.reshape(B, H, D, Sq), 2, 3)
```

```python
import functools

import jax
import jax.numpy as jnp
from jax import lax
from jax.experimental import pallas as pl
from jax.experimental.pallas import tpu as pltpu

_LOG2E = 1.4426950408889634

_QK_LEAD = 2
_PV_LAG = 2
_FIRST = (1, 1, 2)
_LOOKAHEAD = 3
_IN_REGIONS = _LOOKAHEAD + 1
_OUT_REGIONS = 2
_OUT_CHUNK = 5
_RAMP_OUT_AT = 1

_MAIN = (
    ("peq", "col", 4), ("eqp", "col", 4), ("eqp", "row", 1), ("qep", "col", 1),
    ("eqp", "row", 2), ("eqp", "row", 2), ("eqp", "row", 1), ("eqp", "row", 4),
    ("eqp", "col", 1), ("eqp", "row", 1),
)
_RAMP = (
    ((("peq", "col", 1), ("pqe", "row", 1)), 3),
    ((("peq", "row", 4), ("epq", "col", 1), ("qpe", "row", 1),
      ("peq", "col", 1)), 4),
)
_G = len(_MAIN)


def _kernel(q_hbm, k_hbm, v_hbm, o_hbm, qb, kb, vb, ob, s_st, p_st, r_st,
            sin, sout, *, scale, n_heads):
    c = scale * _LOG2E
    G, R, RO, L = _G, _IN_REGIONS, _OUT_REGIONS, _LOOKAHEAD
    dS, dP = _QK_LEAD, _PV_LAG
    D = dS + dP
    n0 = sum(_FIRST)
    nh = n0 + sum(len(seg) * cnt for seg, cnt in _RAMP)
    nmain = (n_heads - nh) // G
    sem_ramp = len(_FIRST)
    sem_main = sem_ramp + sum(cnt for _, cnt in _RAMP)
    sem_last = sem_main + R
    slot_last = nh + R * G
    out0 = nh - D
    out_last = out0 + RO * G

    def in_copy(kind, a, n, slot, si):
        src, dst = ((q_hbm, qb), (k_hbm, kb), (v_hbm, vb))[kind]
        return pltpu.make_async_copy(
            src.at[pl.ds(a, n)], dst.at[pl.ds(slot, n)], sin.at[kind, si])

    def in_group(a, n, slot, si):
        return (in_copy(0, a, n, slot, si), in_copy(1, a, n, slot, si),
                in_copy(2, a - D, n, slot, si))

    def out_copy(a, n, slot, si):
        return pltpu.make_async_copy(
            ob.at[pl.ds(slot, n)], o_hbm.at[pl.ds(a, n)], sout.at[si])

    def qk(slot):
        return lax.dot_general(
            qb[slot], kb[slot], (((0,), (0,)), ((), ())),
            preferred_element_type=jnp.float32)

    def recip(l):
        r = pltpu.reciprocal(l, approx=True)
        return r * (2.0 - l * r)

    def softmax(s, mode="col"):
        m = jnp.max(s, axis=1, keepdims=True)
        p = jnp.exp2((s - m) * c)
        l = jnp.sum(p, axis=1, keepdims=True)
        return p, (recip(l).T if mode == "col" else recip(l.T))

    def pv(slot, oslot, p, r, split=1):
        sq = p.shape[0]
        w = sq if split == 1 else pl.cdiv(sq, 128 * split) * 128
        for q0 in range(0, sq, w):
            q1 = min(q0 + w, sq)
            oT = lax.dot_general(
                vb[slot], p[q0:q1].astype(jnp.bfloat16),
                (((1,), (1,)), ((), ())), preferred_element_type=jnp.float32)
            ob[oslot, :, q0:q1] = (oT * r[:, q0:q1]).astype(ob.dtype)

    def save_state(ss, prs):
        for t, s in enumerate(ss):
            s_st[t] = s
        for t, (p, r) in enumerate(prs):
            p_st[t] = p
            r_st[t] = r

    a, first_at = 0, {}
    for gi, n in enumerate(_FIRST):
        first_at[a] = (in_copy(0, a, n, a, gi), in_copy(1, a, n, a, gi))
        for cp in first_at[a]:
            cp.start()
        a += n
    si = sem_ramp
    for seg, cnt in _RAMP:
        for _ in range(cnt):
            for cp in in_group(a, len(seg), a, si):
                cp.start()
            a, si = a + len(seg), si + 1
    for g in range(min(L, nmain)):
        for cp in in_group(nh + g * G, G, nh + g * G, sem_main + g):
            cp.start()

    S, P = {}, {}
    for h in range(-dS, n0 - dS):
        for cp in first_at.get(h + dS, ()):
            cp.wait()
        if h >= 0:
            P[h] = softmax(S.pop(h))
        S[h + dS] = qk(h + dS)
    save_state([S[h] for h in sorted(S)], [P[h] for h in sorted(P)])

    def segment(steps, a, base, obase, osem, chunk=0, extra=None):
        n = len(steps)
        S = {t - dS: t for t in range(dS)}
        P = {t - D: t for t in range(dP)}

        def step_pv(i):
            j = i - dP
            pr = P.pop(j)
            if isinstance(pr, int):
                pr = (p_st[pr], r_st[pr])
            pv(base + j + D, obase + j + D, *pr, split=steps[i + dS][2])
            done = j + D + 1
            if chunk and done % chunk == 0:
                p0 = done - chunk
                out_copy(a - D + p0, chunk, obase + p0, osem).start()

        def step_softmax(i):
            s = S.pop(i)
            if isinstance(s, int):
                s = s_st[s]
            P[i] = softmax(s, steps[i + dS][1])

        def step_qk(i):
            S[i + dS] = qk(base + i + dS)

        for i in range(-dS, n - dS):
            for piece in steps[i + dS][0]:
                {"p": step_pv, "e": step_softmax, "q": step_qk}[piece](i)
            if extra is not None and i == -1:
                extra()
        save_state(
            [s_st[s] if isinstance(s, int) else s
             for s in (S[h] for h in sorted(S))],
            [(p_st[pr], r_st[pr]) if isinstance(pr, int) else pr
             for pr in (P[h] for h in sorted(P))])

    a0, si0 = n0, sem_ramp
    for seg, cnt in _RAMP:

        def ramp_body(g, carry, seg=seg, a0=a0, si0=si0):
            a = a0 + g * len(seg)
            for cp in in_group(a, len(seg), a, si0 + g):
                cp.wait()
            segment(seg, a, a, a - D, 0)
            return carry

        lax.fori_loop(0, cnt, ramp_body, 0)
        a0, si0 = a0 + len(seg) * cnt, si0 + cnt

    def main_body(g, carry):
        r, ro = g % R, g % RO
        a = nh + g * G
        for cp in in_group(a, G, nh + r * G, sem_main + r):
            cp.wait()

        @pl.when(g >= RO)
        def _():
            out_copy(a - D - RO * G, G, out0 + ro * G, 1 + ro).wait()

        def queue_copies():
            gn = g + L

            @pl.when(gn < nmain)
            def _():
                rn = gn % R
                for cp in in_group(nh + gn * G, G, nh + rn * G, sem_main + rn):
                    cp.start()

            @pl.when(g == _RAMP_OUT_AT)
            def _():
                out_copy(0, nh - D, 0, 0).start()

            @pl.when(gn == nmain)
            def _():
                in_copy(2, n_heads - D, D, slot_last, sem_last).start()

        segment(_MAIN, a, nh + r * G, out0 + ro * G, 1 + ro, _OUT_CHUNK,
                queue_copies)
        return carry

    lax.fori_loop(0, nmain, main_body, 0)

    in_copy(2, n_heads - D, D, slot_last, sem_last).wait()
    P = {}
    for h in range(n_heads - dS, n_heads + dP):
        j = h - dP
        t = j - (n_heads - D)
        pr = P.pop(j) if j in P else (p_st[t], r_st[t])
        pv(slot_last + t, out_last + t, *pr)
        out_copy(j, 1, out_last + t, 1 + RO).start()
        if h < n_heads:
            P[h] = softmax(s_st[h - (n_heads - dS)])

    out_copy(0, nh - D, 0, 0).wait()
    for g in range(max(nmain - RO, 0), nmain):
        out_copy(nh + g * G - D, G, out0 + (g % RO) * G, 1 + g % RO).wait()
    out_copy(n_heads - D, D, out_last, 1 + RO).wait()


@jax.jit
def pallas_standalone__mha_softmax__near_ridge_kernel(
    q: jax.Array,
    k: jax.Array,
    v: jax.Array,
):
    B, H, Sq, D = q.shape
    Sk = k.shape[2]
    n_heads = B * H
    scale = D ** -0.5
    depth = _QK_LEAD + _PV_LAG
    nh = sum(_FIRST) + sum(len(seg) * cnt for seg, cnt in _RAMP)
    assert sum(_FIRST) == depth
    assert (n_heads - nh) % _G == 0
    assert (n_heads - nh) // _G > max(_LOOKAHEAD, _RAMP_OUT_AT)

    qT = jnp.swapaxes(q, 2, 3).reshape(n_heads, D, Sq)
    kT = jnp.swapaxes(k, 2, 3).reshape(n_heads, D, Sk)
    vT = jnp.swapaxes(v, 2, 3).reshape(n_heads, D, Sk)

    n_in = nh + _IN_REGIONS * _G
    n_out = nh + _OUT_REGIONS * _G
    n_sem_in = len(_FIRST) + sum(cnt for _, cnt in _RAMP) + _IN_REGIONS + 1
    oT = pl.pallas_call(
        functools.partial(_kernel, scale=scale, n_heads=n_heads),
        in_specs=[pl.BlockSpec(memory_space=pl.ANY)] * 3,
        out_specs=pl.BlockSpec(memory_space=pl.ANY),
        out_shape=jax.ShapeDtypeStruct((n_heads, D, Sq), q.dtype),
        scratch_shapes=[
            pltpu.VMEM((n_in, D, Sq), q.dtype),
            pltpu.VMEM((n_in, D, Sk), k.dtype),
            pltpu.VMEM((n_in + depth, D, Sk), v.dtype),
            pltpu.VMEM((n_out, D, Sq), q.dtype),
            pltpu.VMEM((_QK_LEAD, Sq, Sk), jnp.float32),
            pltpu.VMEM((_PV_LAG, Sq, Sk), jnp.float32),
            pltpu.VMEM((_PV_LAG, 1, Sq), jnp.float32),
            pltpu.SemaphoreType.DMA((3, n_sem_in)),
            pltpu.SemaphoreType.DMA((2 + _OUT_REGIONS,)),
        ],
        compiler_params=pltpu.CompilerParams(
            vmem_limit_bytes=100 * 1024 * 1024,
            disable_bounds_checks=True,
        ),
    )(qT, kT, vT)
    return jnp.swapaxes(oT.reshape(B, H, D, Sq), 2, 3)
```
